```python
import os as _os
_os.environ.setdefault("JAX_PLATFORMS", "cpu")
import jax
import jax.numpy as jnp

def _softmax(x, axis=-1):
    return jax.nn.softmax(x, axis=axis)
def _gelu(x):
    return jax.nn.gelu(x, approximate=True)
def _silu(x):
    return jax.nn.silu(x)
def _sigmoid(x):
    return jax.nn.sigmoid(x)
def _layernorm(x, axis=-1, eps=1e-5):
    m = jnp.mean(x, axis=axis, keepdims=True)
    v = jnp.var(x, axis=axis, keepdims=True)
    return (x - m) / jnp.sqrt(v + eps)
def _scatter_add(tgt, idx, src, axis=0):
    return tgt.at[idx].add(src)
def _segment_sum(src, seg, n):
    return jax.ops.segment_sum(src, seg, n)
class _Rng:
    def __init__(self, key):
        self._k = key
    def _next(self):
        self._k, sub = jax.random.split(self._k)
        return sub
    def normal(self, shape):
        return jax.random.normal(self._next(), shape, dtype=jnp.bfloat16)
    def randint(self, lo, hi, shape):
        return jax.random.randint(self._next(), shape, lo, hi, dtype=jnp.int32)
    def uniform(self, shape, lo=0.0, hi=1.0):
        return jax.random.uniform(self._next(), shape, jnp.bfloat16, lo, hi)
    def permutation(self, n):
        return jax.random.permutation(self._next(), n)


kernel_name = 'standalone__mha_softmax__near_ridge'

def setup_inputs():
    _rng = _Rng(jax.random.key(int.from_bytes(__import__("os").urandom(4), "little")))
    _w = (lambda a: (lambda t: t.astype(jnp.bfloat16) if jnp.issubdtype(t.dtype, jnp.floating) else t)(jnp.asarray(a)))
    B, H, Sq, Sk, D = 8, 32, 384, 512, 128
    return {
        "q": _w((lambda *s: _rng.normal(s) * 0.4)(B, H, Sq, D)),
        "k": _w((lambda *s: _rng.normal(s) * 0.4)(B, H, Sk, D)),
        "v": _w((lambda *s: _rng.normal(s) * 0.05)(B, H, Sk, D)),
    }

def reference(q, k, v):
    scale = q.shape[-1] ** -0.5
    scores = jnp.einsum("bhqd,bhkd->bhqk", q, k) * scale
    p = _softmax(scores, axis=-1)
    return jnp.einsum("bhqk,bhkd->bhqd", p, v)
```

```python
import functools

import jax
import jax.numpy as jnp
import numpy as np
from jax import lax
from jax.experimental import pallas as pl
from jax.experimental.pallas import tpu as pltpu

_COLS = 16
_GROUP = 4
_WRITE_ROWS = 128
_READ_SEMS = 3
_READ_TAIL = 3
_READ_BOUNDS = (0, 8, 16, 24, 32, 40, 48, 64, 80, 96, 112, 128, 144, 160, 192, 224, 256)
_WRITE_START = 208


def _attend(q, k, v, scale_log2e):
    s = lax.dot_general(
        q, k, (((1,), (1,)), ((), ())), preferred_element_type=jnp.float32
    )
    m = jnp.max(s, axis=-1, keepdims=True)
    p = jnp.exp2((s - m) * scale_log2e)
    l = jnp.sum(p, axis=-1, keepdims=True)
    o = jnp.dot(p.astype(v.dtype), v, preferred_element_type=jnp.float32)
    r = pl.reciprocal(l, approx=True)
    r = r * (2.0 - l * r)
    return o * r


def _kernel(q_hbm, k_hbm, v_hbm, o_hbm, q_buf, k_buf, v_buf, o_buf,
            read_sems, tail_sem, write_sem):
    a_len, s_len, sq, d = q_hbm.shape
    n_heads = a_len * s_len
    bounds = _READ_BOUNDS
    n_chunks = len(bounds) - 1
    scale_log2e = float(d ** -0.5 * np.log2(np.e))

    def heads(ref, lo, hi):
        if lo % a_len == 0 and hi % a_len == 0:
            return ref.at[:, pl.ds(lo // a_len, (hi - lo) // a_len)]
        return ref.at[pl.ds(lo % a_len, hi - lo), pl.ds(lo // a_len, 1)]

    def pieces(lo, hi):
        out = []
        while lo < hi:
            if lo % a_len == 0 and hi - lo >= a_len:
                end = lo + (hi - lo) // a_len * a_len
            else:
                end = min(hi, (lo // a_len + 1) * a_len)
            out.append((lo, end))
            lo = end
        return out

    def reads(i):
        lo, hi = bounds[i], bounds[i + 1]
        v_hi = hi - _READ_TAIL if i == n_chunks - 1 else hi
        sem = read_sems.at[i % _READ_SEMS]
        return [
            pltpu.make_async_copy(heads(src, a, b), heads(dst, a, b), sem)
            for src, dst, end in ((q_hbm, q_buf, hi), (k_hbm, k_buf, hi), (v_hbm, v_buf, v_hi))
            for a, b in pieces(lo, end)
        ]

    def tail_read():
        lo = n_heads - _READ_TAIL
        return pltpu.make_async_copy(
            heads(v_hbm, lo, n_heads), heads(v_buf, lo, n_heads), tail_sem.at[0]
        )

    def start_reads(i):
        for copy in reads(i):
            copy.start()
        if i == n_chunks - 1:
            tail_read().start()

    def start_writes(j):
        for r in range(0, sq, _WRITE_ROWS):
            rows = pl.ds(r, _WRITE_ROWS)
            pltpu.make_async_copy(
                o_buf.at[:, j, rows], o_hbm.at[:, j, rows], write_sem.at[0]
            ).start()

    read_at = [min(bounds[i], _WRITE_START) for i in range(n_chunks)]
    write_at = [max(_WRITE_START, (j + 1) * a_len) for j in range(s_len)]
    stops = sorted(set(read_at) | set(write_at) | {0, n_heads})

    def dma_step(done):
        for i in range(n_chunks):
            if read_at[i] == done:
                for copy in reads(i):
                    copy.wait()
                if i + _READ_SEMS < n_chunks:
                    start_reads(i + _READ_SEMS)
        for j in range(s_len):
            if write_at[j] == done:
                start_writes(j)
        if read_at[-1] == done:
            tail_read().wait()

    def compute(i, carry):
        j = lax.div(i * _GROUP, a_len)
        a0 = lax.rem(i * _GROUP, a_len)
        for g in range(_GROUP):
            a = a0 + g
            out = _attend(q_buf[a, j], k_buf[a, j], v_buf[a, j], scale_log2e)
            o_buf[a, j] = out.astype(o_buf.dtype)
        return carry

    def segment(t, carry):
        lo = hi = jnp.int32(0)
        for n in range(len(stops) - 1):
            lo = jnp.where(t == n, stops[n] // _GROUP, lo)
            hi = jnp.where(t == n, stops[n + 1] // _GROUP, hi)
            pl.when(t == n)(functools.partial(dma_step, stops[n]))
        lax.fori_loop(lo, hi, compute, None)
        return carry

    for i in range(_READ_SEMS):
        start_reads(i)
    lax.fori_loop(0, len(stops) - 1, segment, None)
    dma_step(n_heads)
    pltpu.make_async_copy(o_buf, o_hbm, write_sem.at[0]).wait()


@jax.jit
def pallas_standalone__mha_softmax__near_ridge_kernel(
    q: jax.Array,
    k: jax.Array,
    v: jax.Array,
):
    b, h, sq, d = q.shape
    sk = k.shape[2]
    assert b * h == _READ_BOUNDS[-1]
    a_len = b * h // _COLS
    q_shape = (a_len, _COLS, sq, d)
    kv_shape = (a_len, _COLS, sk, d)
    out = pl.pallas_call(
        _kernel,
        in_specs=[pl.BlockSpec(memory_space=pl.ANY)] * 3,
        out_specs=pl.BlockSpec(memory_space=pl.ANY),
        out_shape=jax.ShapeDtypeStruct(q_shape, q.dtype),
        scratch_shapes=[
            pltpu.VMEM(q_shape, q.dtype),
            pltpu.VMEM(kv_shape, k.dtype),
            pltpu.VMEM(kv_shape, v.dtype),
            pltpu.VMEM(q_shape, q.dtype),
            pltpu.SemaphoreType.DMA((_READ_SEMS,)),
            pltpu.SemaphoreType.DMA((1,)),
            pltpu.SemaphoreType.DMA((1,)),
        ],
        compiler_params=pltpu.CompilerParams(vmem_limit_bytes=126 * 1024 * 1024),
    )(q.reshape(q_shape), k.reshape(kv_shape), v.reshape(kv_shape))
    return out.reshape(q.shape)
```

```python
import jax
import jax.numpy as jnp
import numpy as np
from jax import lax
from jax.experimental import pallas as pl
from jax.experimental.pallas import tpu as pltpu

_COL_HEADS = 8
_WRITE_ROWS = 96
_N_SEMS = 3
_TAIL_HEADS = 3
_READ_BOUNDS = (0, 1, 2, 3, 4, 5, 6, 8, 10, 12, 14, 16, 18, 20, 23, 26, 32)
_WRITES_FIRST = 12
_WRITES_PER_STEP = 5

_N_COLS = _READ_BOUNDS[-1]
_N_CHUNKS = len(_READ_BOUNDS) - 1
_WRITE_STEP = _READ_BOUNDS[-2]
_TAIL_SEM = _N_CHUNKS % _N_SEMS
_WRITE_SEM = (_N_CHUNKS - 1) % _N_SEMS


def _dma_schedule():
    bounds = _READ_BOUNDS
    rows, written = [], 0
    for step in range(_N_COLS):
        awaited = fetched = (0, 0)
        sem = 0
        if step in bounds:
            chunk = bounds.index(step)
            sem = chunk % _N_SEMS
            awaited = bounds[chunk : chunk + 2]
            if chunk + _N_SEMS < _N_CHUNKS:
                fetched = bounds[chunk + _N_SEMS : chunk + _N_SEMS + 2]
        target = written
        if step >= _WRITE_STEP:
            target = _WRITES_FIRST + (step - _WRITE_STEP) * _WRITES_PER_STEP
            target = min(target, step)
        rows.append((*awaited, *fetched, sem, written, target))
        written = target
    return rows


def _attend(q, k, v):
    scale_log2e = float(q.shape[-1] ** -0.5 * np.log2(np.e))
    s = lax.dot_general(
        q, k, (((1,), (1,)), ((), ())), preferred_element_type=jnp.float32
    )
    m = jnp.max(s, axis=-1, keepdims=True)
    p = jnp.exp2((s - m) * scale_log2e)
    l = jnp.sum(p, axis=-1, keepdims=True)
    o = jnp.dot(p.astype(v.dtype), v, preferred_element_type=jnp.float32)
    r = pl.reciprocal(l, approx=True)
    r = r * (2.0 - l * r)
    return o * r


def _for_range(lo, hi, fn):
    def body(i, carry):
        fn(i)
        return carry

    lax.fori_loop(lo, hi, body, None)


def _kernel(q_hbm, k_hbm, v_hbm, o_hbm, q_buf, k_buf, v_buf, o_buf, sems, table):
    last = _N_COLS - 1
    v_heads = _COL_HEADS - _TAIL_HEADS

    def read(src, dst, col, sem, first=0, count=_COL_HEADS):
        return pltpu.make_async_copy(
            src.at[pl.ds(first, count), col],
            dst.at[pl.ds(col * _COL_HEADS + first, count)],
            sems.at[sem],
        )

    def each_read(col, sem, action):
        action(read(q_hbm, q_buf, col, sem))
        action(read(k_hbm, k_buf, col, sem))

        @pl.when(col < last)
        def _():
            action(read(v_hbm, v_buf, col, sem))

        @pl.when(col == last)
        def _():
            action(read(v_hbm, v_buf, last, sem, 0, v_heads))

    def tail_read():
        return read(v_hbm, v_buf, last, _TAIL_SEM, v_heads, _TAIL_HEADS)

    def start_reads(col, sem):
        each_read(col, sem, lambda copy: copy.start())
        pl.when(col == last)(lambda: tail_read().start())

    def each_write(col, action):
        for row in range(0, o_buf.shape[1], _WRITE_ROWS):
            rows = pl.ds(row, _WRITE_ROWS)
            action(pltpu.make_async_copy(
                o_buf.at[pl.ds(col * _COL_HEADS, _COL_HEADS), rows],
                o_hbm.at[:, col, rows],
                sems.at[_WRITE_SEM],
            ))

    def start_writes(col):
        each_write(col, lambda copy: copy.start())

    for chunk in range(_N_SEMS):
        _for_range(
            _READ_BOUNDS[chunk], _READ_BOUNDS[chunk + 1],
            lambda col, sem=chunk: start_reads(col, sem),
        )

    schedule = _dma_schedule()
    width = len(schedule[0])
    for step, row in enumerate(schedule):
        for i, value in enumerate(row):
            table[step * width + i] = jnp.int32(value)

    def step_fn(step):
        wait_lo, wait_hi, read_lo, read_hi, sem, write_lo, write_hi = (
            table[step * width + i] for i in range(width)
        )
        _for_range(wait_lo, wait_hi, lambda col: each_read(col, sem, lambda copy: copy.wait()))
        _for_range(read_lo, read_hi, lambda col: start_reads(col, sem))
        _for_range(write_lo, write_hi, start_writes)
        pl.when(step == _WRITE_STEP)(lambda: tail_read().wait())

        for i in range(_COL_HEADS):
            n = step * _COL_HEADS + i
            o_buf[n] = _attend(q_buf[n], k_buf[n], v_buf[n]).astype(o_buf.dtype)

    _for_range(0, _N_COLS, step_fn)

    _for_range(schedule[-1][-1], _N_COLS, start_writes)
    _for_range(0, _N_COLS, lambda col: each_write(col, lambda copy: copy.wait()))


@jax.jit
def pallas_standalone__mha_softmax__near_ridge_kernel(
    q: jax.Array,
    k: jax.Array,
    v: jax.Array,
):
    b, h, sq, d = q.shape
    assert b * h == _N_COLS * _COL_HEADS and sq % _WRITE_ROWS == 0

    def columns(x):
        return x.reshape(_COL_HEADS, _N_COLS, *x.shape[2:])

    def buffer(x):
        return pltpu.VMEM((b * h, *x.shape[2:]), x.dtype)

    out = pl.pallas_call(
        _kernel,
        in_specs=[pl.BlockSpec(memory_space=pl.ANY)] * 3,
        out_specs=pl.BlockSpec(memory_space=pl.ANY),
        out_shape=jax.ShapeDtypeStruct((_COL_HEADS, _N_COLS, sq, d), q.dtype),
        scratch_shapes=[
            buffer(q),
            buffer(k),
            buffer(v),
            buffer(q),
            pltpu.SemaphoreType.DMA((_N_SEMS,)),
            pltpu.SMEM((_N_COLS * len(_dma_schedule()[0]),), jnp.int32),
        ],
        compiler_params=pltpu.CompilerParams(vmem_limit_bytes=126 * 1024 * 1024),
    )(columns(q), columns(k), columns(v))
    return out.reshape(q.shape)
```

```python
import jax
import jax.numpy as jnp
import numpy as np
from jax import lax
from jax.experimental import pallas as pl
from jax.experimental.pallas import tpu as pltpu

_COL_HEADS = 8
_WRITE_ROWS = 96
_N_SEMS = 3
_TAIL_HEADS = 3
_READ_BOUNDS = (0, 1, 2, 3, 4, 5, 6, 8, 10, 12, 14, 16, 18, 20, 23, 26, 32)
_WRITES_FIRST = 12
_WRITES_PER_STEP = 5

_N_COLS = _READ_BOUNDS[-1]
_N_CHUNKS = len(_READ_BOUNDS) - 1
_WRITE_STEP = _READ_BOUNDS[-2]
_TAIL_STEP = _READ_BOUNDS[_N_CHUNKS - _N_SEMS]
_TAIL_SEM = _N_CHUNKS % _N_SEMS
_WRITE_SEM = (_N_CHUNKS - 1) % _N_SEMS


def _dma_schedule():
    bounds = _READ_BOUNDS
    rows, written = [], 0
    for step in range(_N_COLS):
        awaited = fetched = (0, 0)
        sem = 0
        if step in bounds:
            chunk = bounds.index(step)
            sem = chunk % _N_SEMS
            awaited = bounds[chunk : chunk + 2]
            if chunk + _N_SEMS < _N_CHUNKS:
                fetched = bounds[chunk + _N_SEMS : chunk + _N_SEMS + 2]
        target = written
        if step >= _WRITE_STEP:
            target = _WRITES_FIRST + (step - _WRITE_STEP) * _WRITES_PER_STEP
            target = min(target, step)
        rows.append((*awaited, *fetched, sem, written, target))
        written = target
    return rows


def _attend(q, k, v):
    scale_log2e = float(q.shape[-1] ** -0.5 * np.log2(np.e))
    s = lax.dot_general(
        q, k, (((1,), (1,)), ((), ())), preferred_element_type=jnp.float32
    )
    m = jnp.max(s, axis=-1, keepdims=True)
    p = jnp.exp2((s - m) * scale_log2e)
    l = jnp.sum(p, axis=-1, keepdims=True)
    o = jnp.dot(p.astype(v.dtype), v, preferred_element_type=jnp.float32)
    r = pl.reciprocal(l, approx=True)
    r = r * (2.0 - l * r)
    return o * r


def _for_range(lo, hi, fn):
    def body(i, carry):
        fn(i)
        return carry

    lax.fori_loop(lo, hi, body, None)


def _kernel(q_hbm, k_hbm, v_hbm, o_hbm, q_buf, k_buf, v_buf, o_buf, sems, table):
    last = _N_COLS - 1
    v_heads = _COL_HEADS - _TAIL_HEADS

    def read(src, dst, col, sem, first=0, count=_COL_HEADS):
        return pltpu.make_async_copy(
            src.at[pl.ds(first, count), col],
            dst.at[pl.ds(col * _COL_HEADS + first, count)],
            sems.at[sem],
        )

    def each_read(col, sem, action):
        action(read(q_hbm, q_buf, col, sem))
        action(read(k_hbm, k_buf, col, sem))

        @pl.when(col < last)
        def _():
            action(read(v_hbm, v_buf, col, sem))

        @pl.when(col == last)
        def _():
            action(read(v_hbm, v_buf, last, sem, 0, v_heads))

    def tail_read():
        return read(v_hbm, v_buf, last, _TAIL_SEM, v_heads, _TAIL_HEADS)

    def start_reads(col, sem):
        each_read(col, sem, lambda copy: copy.start())

    def wait_reads(col, sem):
        each_read(col, sem, lambda copy: copy.wait())

    def each_write(col, action):
        for row in range(0, o_buf.shape[1], _WRITE_ROWS):
            rows = pl.ds(row, _WRITE_ROWS)
            action(pltpu.make_async_copy(
                o_buf.at[pl.ds(col * _COL_HEADS, _COL_HEADS), rows],
                o_hbm.at[:, col, rows],
                sems.at[_WRITE_SEM],
            ))

    def start_writes(col):
        each_write(col, lambda copy: copy.start())

    for chunk in range(_N_SEMS):
        _for_range(
            _READ_BOUNDS[chunk], _READ_BOUNDS[chunk + 1],
            lambda col, sem=chunk: start_reads(col, sem),
        )

    schedule = _dma_schedule()
    width = len(schedule[0])
    for step, row in enumerate(schedule):
        for i, value in enumerate(row):
            table[step * width + i] = jnp.int32(value)

    def step_fn(step):
        wait_lo, wait_hi, read_lo, read_hi, sem, write_lo, write_hi = (
            table[step * width + i] for i in range(width)
        )
        _for_range(wait_lo, wait_hi, lambda col: wait_reads(col, sem))
        _for_range(read_lo, read_hi, lambda col: start_reads(col, sem))
        pl.when(step == _TAIL_STEP)(lambda: tail_read().start())
        _for_range(write_lo, write_hi, start_writes)
        pl.when(step == _WRITE_STEP)(lambda: tail_read().wait())

        for i in range(_COL_HEADS):
            n = step * _COL_HEADS + i
            o_buf[n] = _attend(q_buf[n], k_buf[n], v_buf[n]).astype(o_buf.dtype)

    _for_range(0, _N_COLS, step_fn)

    _for_range(schedule[-1][-1], _N_COLS, start_writes)
    _for_range(0, _N_COLS, lambda col: each_write(col, lambda copy: copy.wait()))


@jax.jit
def pallas_standalone__mha_softmax__near_ridge_kernel(
    q: jax.Array,
    k: jax.Array,
    v: jax.Array,
):
    b, h, sq, d = q.shape
    assert b * h == _N_COLS * _COL_HEADS and sq % _WRITE_ROWS == 0

    def columns(x):
        return x.reshape(_COL_HEADS, _N_COLS, *x.shape[2:])

    def buffer(x):
        return pltpu.VMEM((b * h, *x.shape[2:]), x.dtype)

    out = pl.pallas_call(
        _kernel,
        in_specs=[pl.BlockSpec(memory_space=pl.ANY)] * 3,
        out_specs=pl.BlockSpec(memory_space=pl.ANY),
        out_shape=jax.ShapeDtypeStruct((_COL_HEADS, _N_COLS, sq, d), q.dtype),
        scratch_shapes=[
            buffer(q),
            buffer(k),
            buffer(v),
            buffer(q),
            pltpu.SemaphoreType.DMA((_N_SEMS,)),
            pltpu.SMEM((_N_COLS * len(_dma_schedule()[0]),), jnp.int32),
        ],
        compiler_params=pltpu.CompilerParams(vmem_limit_bytes=126 * 1024 * 1024),
    )(columns(q), columns(k), columns(v))
    return out.reshape(q.shape)
```
